```python
import os as _os
_os.environ.setdefault("JAX_PLATFORMS", "cpu")
import jax
import jax.numpy as jnp

def _softmax(x, axis=-1):
    return jax.nn.softmax(x, axis=axis)
def _gelu(x):
    return jax.nn.gelu(x, approximate=True)
def _silu(x):
    return jax.nn.silu(x)
def _sigmoid(x):
    return jax.nn.sigmoid(x)
def _layernorm(x, axis=-1, eps=1e-5):
    m = jnp.mean(x, axis=axis, keepdims=True)
    v = jnp.var(x, axis=axis, keepdims=True)
    return (x - m) / jnp.sqrt(v + eps)
def _scatter_add(tgt, idx, src, axis=0):
    return tgt.at[idx].add(src)
def _segment_sum(src, seg, n):
    return jax.ops.segment_sum(src, seg, n)
class _Rng:
    def __init__(self, key):
        self._k = key
    def _next(self):
        self._k, sub = jax.random.split(self._k)
        return sub
    def normal(self, shape):
        return jax.random.normal(self._next(), shape, dtype=jnp.bfloat16)
    def randint(self, lo, hi, shape):
        return jax.random.randint(self._next(), shape, lo, hi, dtype=jnp.int32)
    def uniform(self, shape, lo=0.0, hi=1.0):
        return jax.random.uniform(self._next(), shape, jnp.bfloat16, lo, hi)
    def permutation(self, n):
        return jax.random.permutation(self._next(), n)


kernel_name = 'standalone__channel_attn_cbam__vision'

def setup_inputs():
    _rng = _Rng(jax.random.key(int.from_bytes(__import__("os").urandom(4), "little")))
    _w = (lambda a: (lambda t: t.astype(jnp.bfloat16) if jnp.issubdtype(t.dtype, jnp.floating) else t)(jnp.asarray(a)))
    H = W = 384
    C = 192
    r = max(C // 4, 1)
    return {
        "x": _w((lambda *s: _rng.normal(s) * 0.2)(1, H, W, C) + (lambda *s: _rng.normal(s) * 0.2)(1, 1, 1, C) * 2.0),
        "w1": _w((lambda *s: _rng.normal(s) * 0.2)(C, r)),
        "w2": _w((lambda *s: _rng.normal(s) * 0.2)(r, C)),
    }

def reference(x, w1, w2):
    B, H, W, C = x.shape
    xf = x.reshape(B, H * W, C)
    gap = jnp.mean(xf, 1)
    gmp = jnp.amax(xf, 1)
    h_a = gap @ w1
    h_a = h_a * (lambda x, dt: x.astype(dt))(h_a > 0, h_a.dtype)
    h_m = gmp @ w1
    h_m = h_m * (lambda x, dt: x.astype(dt))(h_m > 0, h_m.dtype)
    scale = _sigmoid(h_a @ w2 + h_m @ w2)
    return x * scale[:, None, None, :]
```

```python
import jax
import jax.numpy as jnp
from jax import lax
import jax.experimental.pallas as pl
import jax.experimental.pallas.tpu as pltpu

H, W, C, R = 384, 384, 192, 48
LANES = 128
SUB = 8
WT = W // LANES
CB = C // SUB
TPH = CB * WT
RPH = TPH * SUB
NT = H * TPH
NROWS = NT * SUB

READ_CHUNKS = (256, 96, 24, 6, 2)
GRP = 4
NGRP = CB // GRP
GROWS = GRP * WT * SUB

SLAB = 256
NSLAB = NT // SLAB
RUN = 16
NRUN = SLAB // RUN
FIRST_SPLIT = (4, 20, 84)
TAB_TILES = TPH + RUN


def _kernel(x_hbm, w1t_hbm, w2_hbm, o_hbm,
            buf, w1t_v, w2_v, w2t_v, sum_v, max_v, tab,
            rsem, wsem, psem):
    cw1 = pltpu.make_async_copy(w1t_hbm, w1t_v, psem.at[0])
    cw2 = pltpu.make_async_copy(w2_hbm, w2_v, psem.at[1])
    rcopies = []
    h0 = 0
    for k, nh in enumerate(READ_CHUNKS):
        sl = pl.ds(h0 * RPH, nh * RPH)
        c = pltpu.make_async_copy(x_hbm.at[sl], buf.at[sl], rsem.at[k])
        c.start(priority=1)
        if k == 0:
            cw1.start()
            cw2.start()
        rcopies.append((c, h0, nh))
        h0 += nh

    sum_v[...] = jnp.zeros(sum_v.shape, jnp.float32)
    max_v[...] = jnp.full(max_v.shape, -jnp.inf, jnp.float32)

    def accum(row, s, m):
        v = buf[pl.ds(row, GROWS), :].astype(jnp.float32)
        v = v.reshape(GRP, WT, SUB, LANES)
        s = s + ((v[:, 0] + v[:, 1]) + v[:, 2])
        m = jnp.maximum(m, jnp.maximum(jnp.maximum(v[:, 0], v[:, 1]), v[:, 2]))
        return s, m

    for k, (c, h0, nh) in enumerate(rcopies):
        c.wait()
        if k == 0:
            cw1.wait()
            cw2.wait()
            w2t_v[...] = w2_v[...].astype(jnp.float32).T.astype(jnp.bfloat16)

        def group(g, carry, h0=h0, nh=nh):
            gs = pl.ds(g * GRP, GRP)

            def body(h, sm):
                row = pl.multiple_of(h * RPH + g * GROWS, 32)
                return accum(row, *sm)

            s, m = lax.fori_loop(h0, h0 + nh, body, (sum_v[gs], max_v[gs]),
                                 unroll=2)
            sum_v[gs] = s
            max_v[gs] = m
            return carry

        lax.fori_loop(0, NGRP, group, 0)

    ssum = jnp.sum(sum_v[...].reshape(C, LANES), axis=1, keepdims=True)
    smax = jnp.max(max_v[...].reshape(C, LANES), axis=1, keepdims=True)
    gap = ssum / float(H * W)
    lane = lax.broadcasted_iota(jnp.int32, (C, LANES), 1)
    desc = jnp.where(lane < LANES // 2, gap, smax).astype(jnp.bfloat16)
    hid = jnp.dot(w1t_v[...], desc, preferred_element_type=jnp.float32)
    hid = hid.astype(jnp.bfloat16).astype(jnp.float32)
    hid = (hid * (hid > 0).astype(jnp.float32)).astype(jnp.bfloat16)
    o = jnp.dot(w2t_v[...], hid, preferred_element_type=jnp.float32)
    o = o.astype(jnp.bfloat16).astype(jnp.float32)
    z = (o + pltpu.roll(o, LANES // 2, 1)).astype(jnp.bfloat16).astype(jnp.float32)
    scale = jax.nn.sigmoid(z).astype(jnp.bfloat16).astype(jnp.float32)
    scale = scale.reshape(CB, SUB, LANES)
    for t in range(TAB_TILES):
        tab[t] = scale[(t % TPH) // WT]

    buf3 = buf.reshape(NSLAB, SLAB * SUB, LANES)

    def scale_run(j, a):
        t0 = a * SLAB + j * RUN
        row = pl.multiple_of(t0 * SUB, RUN * SUB)
        ph = lax.rem(t0, TPH)
        sc = tab[pl.ds(ph, RUN)].reshape(RUN * SUB, LANES)
        v = buf[pl.ds(row, RUN * SUB), :].astype(jnp.float32)
        buf[pl.ds(row, RUN * SUB), :] = (v * sc).astype(jnp.bfloat16)

    wcopies = []

    def emit(j, a0, na):
        def body(a, carry):
            scale_run(j, a)
            return carry

        lax.fori_loop(a0, a0 + na, body, 0, unroll=2)
        rs = pl.ds(j * RUN * SUB, RUN * SUB)
        c = pltpu.make_async_copy(buf3.at[pl.ds(a0, na), rs, :],
                                  o_hbm.at[pl.ds(a0, na), rs, :],
                                  wsem.at[len(wcopies)])
        c.start()
        wcopies.append(c)

    a0 = 0
    for na in FIRST_SPLIT:
        emit(0, a0, na)
        a0 += na
    for j in range(1, NRUN):
        emit(j, 0, NSLAB)
    for c in wcopies:
        c.wait()


@jax.jit
def pallas_standalone__channel_attn_cbam__vision_kernel(
    x: jax.Array,
    w1: jax.Array,
    w2: jax.Array,
):
    assert x.shape == (1, H, W, C) and w1.shape == (C, R) and w2.shape == (R, C)
    xt = jnp.transpose(x, (0, 1, 3, 2)).reshape(H, CB, SUB, WT, LANES)
    xt = jnp.transpose(xt, (0, 1, 3, 2, 4)).reshape(NROWS, LANES)

    n_w = len(FIRST_SPLIT) + NRUN - 1
    out = pl.pallas_call(
        _kernel,
        out_shape=jax.ShapeDtypeStruct((NSLAB, SLAB * SUB, LANES), x.dtype),
        in_specs=[pl.BlockSpec(memory_space=pl.ANY)] * 3,
        out_specs=pl.BlockSpec(memory_space=pl.ANY),
        scratch_shapes=[
            pltpu.VMEM((NROWS, LANES), jnp.bfloat16),
            pltpu.VMEM((R, C), jnp.bfloat16),
            pltpu.VMEM((R, C), jnp.bfloat16),
            pltpu.VMEM((C, R), jnp.bfloat16),
            pltpu.VMEM((CB, SUB, LANES), jnp.float32),
            pltpu.VMEM((CB, SUB, LANES), jnp.float32),
            pltpu.VMEM((TAB_TILES, SUB, LANES), jnp.float32),
            pltpu.SemaphoreType.DMA((len(READ_CHUNKS),)),
            pltpu.SemaphoreType.DMA((n_w,)),
            pltpu.SemaphoreType.DMA((2,)),
        ],
        compiler_params=pltpu.CompilerParams(vmem_limit_bytes=96 * 1024 * 1024),
    )(xt, w1.T, w2)

    out = out.reshape(H, CB, WT, SUB, LANES)
    out = jnp.transpose(out, (0, 1, 3, 2, 4)).reshape(1, H, C, W)
    return jnp.transpose(out, (0, 1, 3, 2))
```

```python
import jax
import jax.numpy as jnp
from jax import lax
import jax.experimental.pallas as pl
import jax.experimental.pallas.tpu as pltpu

F32, BF16 = jnp.float32, jnp.bfloat16

H, W, C, R = 384, 384, 192, 48
LANES, SUB = 128, 8
HALF = LANES // 2
WT = W // LANES
CB = C // SUB
TPH = CB * WT
RPH = TPH * SUB
CROWS = WT * SUB
NT = H * TPH

BULK = (272, 72, 24)
EARLY_TAIL = (8, 4, 2, 1, 1)
LATE_TAIL = (12, 3, 1)
LATE = 4
EARLY = CB - LATE
GRP = 4
UNROLL = 8

NS = 6
SLAB = 512
NSLAB = NT // SLAB
RUN = 6
NPER = SLAB // TPH
PREM = SLAB - NPER * TPH
GSHIFT = (NS * PREM) % TPH
TABN = max((g * GSHIFT) % TPH for g in range(NSLAB // NS)) + (NS - 1) * PREM + TPH
AH = NPER
AROWS = NS * AH
AREM = (NS * SLAB - AROWS * TPH) // WT
HEAD = 2
AREST = (4, 6, 6, 6)


def _rnd(v):
    return v.astype(BF16).astype(F32)


def _kernel(x_hbm, w1t_hbm, w2_hbm, o_hbm,
            buf, w1t_v, w2_v, w1d_v, w2d_v, sum_v, max_v, scale_v, tab,
            rsem, wsem, psem):
    pieces = []

    def piece(h0, nh, c0, nc):
        rs = pl.ds(c0 * CROWS, nc * CROWS)
        hs = pl.ds(h0, nh)
        c = pltpu.make_async_copy(x_hbm.at[hs, rs], buf.at[hs, rs], rsem.at[len(pieces)])
        c.start(priority=1)
        pieces.append(c)
        return c, h0, nh

    def schedule(h0, sizes, c0, nc):
        out = []
        for nh in sizes:
            out.append(piece(h0, nh, c0, nc))
            h0 += nh
        return out

    bulk = schedule(0, BULK, 0, CB)
    early = schedule(sum(BULK), EARLY_TAIL, 0, EARLY)
    late = schedule(sum(BULK), LATE_TAIL, EARLY, LATE)
    cw1 = pltpu.make_async_copy(w1t_hbm, w1t_v, psem.at[0])
    cw2 = pltpu.make_async_copy(w2_hbm, w2_v, psem.at[1])
    cw1.start()
    cw2.start()

    sum_v[...] = jnp.zeros(sum_v.shape, F32)
    max_v[...] = jnp.full(max_v.shape, -jnp.inf, F32)

    cw1.wait()
    cw2.wait()
    zpad = jnp.zeros((HALF - R, C), F32)
    for src, dst in ((w1t_v, w1d_v), (w2_v, w2d_v)):
        w = src[...].astype(F32)
        dst[...] = jnp.concatenate([w, zpad, w, zpad], axis=0).T.reshape(CB, SUB, LANES)

    def accum(h, nh, c0, nc, s, m):
        for i in range(nh):
            v = buf[h + i, pl.ds(c0 * CROWS, nc * CROWS), :].astype(F32)
            v = v.reshape(nc, WT, SUB, LANES)
            s = s + ((v[:, 0] + v[:, 1]) + v[:, 2])
            m = jnp.maximum(m, jnp.maximum(jnp.maximum(v[:, 0], v[:, 1]), v[:, 2]))
        return s, m

    def reduce_rows(h0, nh, nc):
        for g0 in range(0, nc, GRP):
            gs = pl.ds(g0, GRP)
            if nh <= UNROLL:
                s, m = accum(h0, nh, g0, GRP, sum_v[gs], max_v[gs])
            else:
                s, m = lax.fori_loop(
                    0, nh // UNROLL,
                    lambda i, sm, g0=g0: accum(h0 + i * UNROLL, UNROLL, g0, GRP, *sm),
                    (sum_v[gs], max_v[gs]))
            sum_v[gs] = s
            max_v[gs] = m

    lane = lax.broadcasted_iota(jnp.int32, (1, LANES), 1)

    def layer1(s, m, c0, nc):
        gap = _rnd(jnp.sum(s, axis=2, keepdims=True) * (1.0 / (H * W)))
        gmp = jnp.max(m, axis=2, keepdims=True)
        desc = jnp.where(lane[None] < HALF, gap, gmp)
        return jnp.sum(desc * w1d_v[pl.ds(c0, nc)], axis=0)

    for c, h0, nh in bulk:
        c.wait()
        reduce_rows(h0, nh, CB)
    for c, h0, nh in early[:-1]:
        c.wait()
        reduce_rows(h0, nh, EARLY)
    c, h0, nh = early[-1]
    c.wait()
    es = pl.ds(0, EARLY)
    part = layer1(*accum(h0, nh, 0, EARLY, sum_v[es], max_v[es]), 0, EARLY)
    ls = pl.ds(EARLY, LATE)
    s, m = sum_v[ls], max_v[ls]
    for c, h0, nh in late:
        c.wait()
        s, m = accum(h0, nh, EARLY, LATE, s, m)

    hid = _rnd(jnp.sum(part + layer1(s, m, EARLY, LATE), axis=0, keepdims=True))
    hid = hid * (hid > 0).astype(F32)
    hid_a = jnp.where(lane < R, hid, 0.0)
    hid_m = jnp.where((lane >= HALF) & (lane < HALF + R), hid, 0.0)

    def scales(c0, nc):
        w2d = w2d_v[pl.ds(c0, nc)]
        za = _rnd(jnp.sum(w2d * hid_a[None], axis=2, keepdims=True))
        zm = _rnd(jnp.sum(w2d * hid_m[None], axis=2, keepdims=True))
        sc = _rnd(jax.nn.sigmoid(_rnd(za + zm)))
        return jnp.broadcast_to(sc, (nc, SUB, LANES))

    buf_a = buf.at[pl.ds(0, AROWS)].reshape(NS, AH, RPH, LANES)
    out_a = o_hbm.at[pl.ds(0, AROWS)].reshape(NS, AH, RPH, LANES)
    buf_b = buf.reshape(NSLAB, SLAB * SUB, LANES)
    out_b = o_hbm.reshape(NSLAB, SLAB * SUB, LANES)

    def run_a(h, c0, nc, sc):
        rs = pl.ds(c0 * CROWS, nc * CROWS)
        v = buf_a[:, h, rs, :].astype(F32).reshape(NS, nc, WT, SUB, LANES)
        buf_a[:, h, rs, :] = (v * sc[None, :, None]).reshape(NS, nc * CROWS, LANES).astype(BF16)
        pltpu.make_async_copy(buf_a.at[:, h, rs, :], out_a.at[:, h, rs, :], wsem).start()

    sc_head = scales(0, HEAD)
    scale_v[pl.ds(0, HEAD)] = sc_head
    run_a(0, 0, HEAD, sc_head)

    def head_rows(h, carry):
        run_a(h, 0, HEAD, sc_head)
        return carry

    lax.fori_loop(1, AH, head_rows, 0)
    scale_v[pl.ds(HEAD, CB - HEAD)] = scales(HEAD, CB - HEAD)

    def rest_rows(h, carry):
        c0 = HEAD
        for nc in AREST:
            run_a(h, c0, nc, scale_v[pl.ds(c0, nc)])
            c0 += nc
        return carry

    lax.fori_loop(0, AH, rest_rows, 0)

    rs = pl.ds(0, AREM * CROWS)
    v = buf[AROWS, rs, :].astype(F32).reshape(AREM, WT, SUB, LANES)
    v = v * scale_v[pl.ds(0, AREM)][:, None]
    buf[AROWS, rs, :] = v.reshape(AREM * CROWS, LANES).astype(BF16)
    pltpu.make_async_copy(buf.at[AROWS, rs, :], o_hbm.at[AROWS, rs, :], wsem).start()

    for t in range(TABN):
        tab[t] = scale_v[(t % TPH) // WT]

    def run_b(s0, phase, row0, t, n):
        ss = pl.ds(s0, NS)
        rs = pl.ds(pl.multiple_of(row0 + t * SUB, 2 * SUB), n * SUB)
        sc = jnp.stack([tab[pl.ds(phase + (a * PREM + t), n)] for a in range(NS)])
        v = buf_b[ss, rs, :].astype(F32).reshape(NS, n, SUB, LANES)
        buf_b[ss, rs, :] = (v * sc).reshape(NS, n * SUB, LANES).astype(BF16)
        pltpu.make_async_copy(buf_b.at[ss, rs, :], out_b.at[ss, rs, :], wsem).start()

    def slab_group(g, phase):
        s0 = g * NS

        def period(j, carry):
            for t in range(0, TPH, RUN):
                run_b(s0, phase, j * RPH, t, RUN)
            return carry

        lax.fori_loop(0, NPER, period, 0)
        run_b(s0, phase, NPER * RPH, 0, PREM)
        phase = phase + GSHIFT
        return jnp.where(phase >= TPH, phase - TPH, phase)

    lax.fori_loop(1, NSLAB // NS, slab_group, jnp.int32(GSHIFT))

    pltpu.make_async_copy(buf, o_hbm, wsem).wait()


@jax.jit
def pallas_standalone__channel_attn_cbam__vision_kernel(
    x: jax.Array,
    w1: jax.Array,
    w2: jax.Array,
):
    assert x.shape == (1, H, W, C) and w1.shape == (C, R) and w2.shape == (R, C)
    xt = jnp.transpose(x, (0, 1, 3, 2)).reshape(H, CB, SUB, WT, LANES)
    xt = jnp.transpose(xt, (0, 1, 3, 2, 4)).reshape(H, RPH, LANES)

    stat = pltpu.VMEM((CB, SUB, LANES), F32)
    out = pl.pallas_call(
        _kernel,
        out_shape=jax.ShapeDtypeStruct((H, RPH, LANES), x.dtype),
        in_specs=[pl.BlockSpec(memory_space=pl.ANY)] * 3,
        out_specs=pl.BlockSpec(memory_space=pl.ANY),
        scratch_shapes=[
            pltpu.VMEM((H, RPH, LANES), BF16),
            pltpu.VMEM((R, C), BF16),
            pltpu.VMEM((R, C), BF16),
            stat, stat,
            stat, stat,
            stat,
            pltpu.VMEM((TABN, SUB, LANES), F32),
            pltpu.SemaphoreType.DMA((len(BULK) + len(EARLY_TAIL) + len(LATE_TAIL),)),
            pltpu.SemaphoreType.DMA(()),
            pltpu.SemaphoreType.DMA((2,)),
        ],
        compiler_params=pltpu.CompilerParams(
            vmem_limit_bytes=96 * 1024 * 1024,
            disable_semaphore_checks=True,
        ),
    )(xt, w1.T, w2)

    out = out.reshape(H, CB, WT, SUB, LANES)
    out = jnp.transpose(out, (0, 1, 3, 2, 4)).reshape(1, H, C, W)
    return jnp.transpose(out, (0, 1, 3, 2))
```

```python
import jax
import jax.numpy as jnp
from jax import lax
import jax.experimental.pallas as pl
import jax.experimental.pallas.tpu as pltpu

F32, BF16 = jnp.float32, jnp.bfloat16

H, W, C, R = 384, 384, 192, 48
LANES, SUB = 128, 8
HALF = LANES // 2
WT = W // LANES
CB = C // SUB
TPH = CB * WT
RPH = TPH * SUB
CROWS = WT * SUB
NT = H * TPH

BULK = (272, 72, 24)
EARLY_TAIL = (8, 4, 2, 1, 1)
LATE_TAIL = (12, 3, 1)
LATE = 4
EARLY = CB - LATE
GRP = 4
UNROLL = 8

NS = 6
SLAB = 512
NSLAB = NT // SLAB
RUN = 6
NPER = SLAB // TPH
PREM = SLAB - NPER * TPH
GSHIFT = (NS * PREM) % TPH
TABN = max((g * GSHIFT) % TPH for g in range(NSLAB // NS)) + (NS - 1) * PREM + TPH
NA, AH = 7, 6
AROWS = NA * AH
AREM = (NS * SLAB - AROWS * TPH) // WT
HEAD = 2
AREST = (4, 6, 6, 6)


def _rnd(v):
    return v.astype(BF16).astype(F32)


def _kernel(x_hbm, w1t_hbm, w2_hbm, o_hbm,
            buf, w1t_v, w2_v, w1d_v, w2d_v, sum_v, max_v, scale_v, tab,
            rsem, wsem, psem):
    pieces = []

    def piece(h0, nh, c0, nc):
        rs = pl.ds(c0 * CROWS, nc * CROWS)
        hs = pl.ds(h0, nh)
        c = pltpu.make_async_copy(x_hbm.at[hs, rs], buf.at[hs, rs], rsem.at[len(pieces)])
        c.start(priority=1)
        pieces.append(c)
        return c, h0, nh

    def schedule(h0, sizes, c0, nc):
        out = []
        for nh in sizes:
            out.append(piece(h0, nh, c0, nc))
            h0 += nh
        return out

    bulk = schedule(0, BULK, 0, CB)
    early = schedule(sum(BULK), EARLY_TAIL, 0, EARLY)
    late = schedule(sum(BULK), LATE_TAIL, EARLY, LATE)
    cw1 = pltpu.make_async_copy(w1t_hbm, w1t_v, psem.at[0])
    cw2 = pltpu.make_async_copy(w2_hbm, w2_v, psem.at[1])
    cw1.start()
    cw2.start()

    sum_v[...] = jnp.zeros(sum_v.shape, F32)
    max_v[...] = jnp.full(max_v.shape, -jnp.inf, F32)

    cw1.wait()
    cw2.wait()
    zpad = jnp.zeros((HALF - R, C), F32)
    for src, dst in ((w1t_v, w1d_v), (w2_v, w2d_v)):
        w = src[...].astype(F32)
        dst[...] = jnp.concatenate([w, zpad, w, zpad], axis=0).T.reshape(CB, SUB, LANES)

    def accum(h, nh, c0, nc, s, m):
        for i in range(nh):
            v = buf[h + i, pl.ds(c0 * CROWS, nc * CROWS), :].astype(F32)
            v = v.reshape(nc, WT, SUB, LANES)
            s = s + ((v[:, 0] + v[:, 1]) + v[:, 2])
            m = jnp.maximum(m, jnp.maximum(jnp.maximum(v[:, 0], v[:, 1]), v[:, 2]))
        return s, m

    def reduce_rows(h0, nh, nc):
        for g0 in range(0, nc, GRP):
            gs = pl.ds(g0, GRP)
            if nh <= UNROLL:
                s, m = accum(h0, nh, g0, GRP, sum_v[gs], max_v[gs])
            else:
                s, m = lax.fori_loop(
                    0, nh // UNROLL,
                    lambda i, sm, g0=g0: accum(h0 + i * UNROLL, UNROLL, g0, GRP, *sm),
                    (sum_v[gs], max_v[gs]))
            sum_v[gs] = s
            max_v[gs] = m

    lane = lax.broadcasted_iota(jnp.int32, (1, LANES), 1)

    def layer1(s, m, c0, nc):
        gap = _rnd(jnp.sum(s, axis=2, keepdims=True) * (1.0 / (H * W)))
        gmp = jnp.max(m, axis=2, keepdims=True)
        desc = jnp.where(lane[None] < HALF, gap, gmp)
        return jnp.sum(desc * w1d_v[pl.ds(c0, nc)], axis=0)

    for c, h0, nh in bulk:
        c.wait()
        reduce_rows(h0, nh, CB)
    for c, h0, nh in early[:-1]:
        c.wait()
        reduce_rows(h0, nh, EARLY)
    c, h0, nh = early[-1]
    c.wait()
    es = pl.ds(0, EARLY)
    part = layer1(*accum(h0, nh, 0, EARLY, sum_v[es], max_v[es]), 0, EARLY)
    ls = pl.ds(EARLY, LATE)
    s, m = sum_v[ls], max_v[ls]
    for c, h0, nh in late:
        c.wait()
        s, m = accum(h0, nh, EARLY, LATE, s, m)

    hid = _rnd(jnp.sum(part + layer1(s, m, EARLY, LATE), axis=0, keepdims=True))
    hid = hid * (hid > 0).astype(F32)
    hid_a = jnp.where(lane < R, hid, 0.0)
    hid_m = jnp.where((lane >= HALF) & (lane < HALF + R), hid, 0.0)

    def scales(c0, nc):
        w2d = w2d_v[pl.ds(c0, nc)]
        za = _rnd(jnp.sum(w2d * hid_a[None], axis=2, keepdims=True))
        zm = _rnd(jnp.sum(w2d * hid_m[None], axis=2, keepdims=True))
        sc = _rnd(jax.nn.sigmoid(_rnd(za + zm)))
        return jnp.broadcast_to(sc, (nc, SUB, LANES))

    buf_a = buf.reshape(H // AH, AH, RPH, LANES)
    out_a = o_hbm.reshape(H // AH, AH, RPH, LANES)
    buf_b = buf.reshape(NSLAB, SLAB * SUB, LANES)
    out_b = o_hbm.reshape(NSLAB, SLAB * SUB, LANES)

    def run_a(h, c0, nc, sc):
        ss = pl.ds(0, NA)
        rs = pl.ds(c0 * CROWS, nc * CROWS)
        v = buf_a[ss, h, rs, :].astype(F32).reshape(NA, nc, WT, SUB, LANES)
        buf_a[ss, h, rs, :] = (v * sc[None, :, None]).reshape(NA, nc * CROWS, LANES).astype(BF16)
        pltpu.make_async_copy(buf_a.at[ss, h, rs, :], out_a.at[ss, h, rs, :], wsem).start()

    sc_head = scales(0, HEAD)
    scale_v[pl.ds(0, HEAD)] = sc_head
    run_a(0, 0, HEAD, sc_head)

    def head_rows(h, carry):
        run_a(h, 0, HEAD, sc_head)
        return carry

    lax.fori_loop(1, AH, head_rows, 0)
    scale_v[pl.ds(HEAD, CB - HEAD)] = scales(HEAD, CB - HEAD)

    def rest_rows(h, carry):
        c0 = HEAD
        for nc in AREST:
            run_a(h, c0, nc, scale_v[pl.ds(c0, nc)])
            c0 += nc
        return carry

    lax.fori_loop(0, AH, rest_rows, 0)

    rs = pl.ds(0, AREM * CROWS)
    v = buf[AROWS, rs, :].astype(F32).reshape(AREM, WT, SUB, LANES)
    v = v * scale_v[pl.ds(0, AREM)][:, None]
    buf[AROWS, rs, :] = v.reshape(AREM * CROWS, LANES).astype(BF16)
    pltpu.make_async_copy(buf.at[AROWS, rs, :], o_hbm.at[AROWS, rs, :], wsem).start()

    for t in range(TABN):
        tab[t] = scale_v[(t % TPH) // WT]

    def run_b(s0, phase, row0, t, n):
        ss = pl.ds(s0, NS)
        rs = pl.ds(pl.multiple_of(row0 + t * SUB, 2 * SUB), n * SUB)
        sc = jnp.stack([tab[pl.ds(phase + (a * PREM + t), n)] for a in range(NS)])
        v = buf_b[ss, rs, :].astype(F32).reshape(NS, n, SUB, LANES)
        buf_b[ss, rs, :] = (v * sc).reshape(NS, n * SUB, LANES).astype(BF16)
        pltpu.make_async_copy(buf_b.at[ss, rs, :], out_b.at[ss, rs, :], wsem).start()

    def slab_group(g, phase):
        s0 = g * NS

        def period(j, carry):
            for t in range(0, TPH, RUN):
                run_b(s0, phase, j * RPH, t, RUN)
            return carry

        lax.fori_loop(0, NPER, period, 0)
        run_b(s0, phase, NPER * RPH, 0, PREM)
        phase = phase + GSHIFT
        return jnp.where(phase >= TPH, phase - TPH, phase)

    lax.fori_loop(1, NSLAB // NS, slab_group, jnp.int32(GSHIFT))

    pltpu.make_async_copy(buf, o_hbm, wsem).wait()


@jax.jit
def pallas_standalone__channel_attn_cbam__vision_kernel(
    x: jax.Array,
    w1: jax.Array,
    w2: jax.Array,
):
    assert x.shape == (1, H, W, C) and w1.shape == (C, R) and w2.shape == (R, C)
    xt = jnp.transpose(x, (0, 1, 3, 2)).reshape(H, CB, SUB, WT, LANES)
    xt = jnp.transpose(xt, (0, 1, 3, 2, 4)).reshape(H, RPH, LANES)

    stat = pltpu.VMEM((CB, SUB, LANES), F32)
    out = pl.pallas_call(
        _kernel,
        out_shape=jax.ShapeDtypeStruct((H, RPH, LANES), x.dtype),
        in_specs=[pl.BlockSpec(memory_space=pl.ANY)] * 3,
        out_specs=pl.BlockSpec(memory_space=pl.ANY),
        scratch_shapes=[
            pltpu.VMEM((H, RPH, LANES), BF16),
            pltpu.VMEM((R, C), BF16),
            pltpu.VMEM((R, C), BF16),
            stat, stat,
            stat, stat,
            stat,
            pltpu.VMEM((TABN, SUB, LANES), F32),
            pltpu.SemaphoreType.DMA((len(BULK) + len(EARLY_TAIL) + len(LATE_TAIL),)),
            pltpu.SemaphoreType.DMA(()),
            pltpu.SemaphoreType.DMA((2,)),
        ],
        compiler_params=pltpu.CompilerParams(
            vmem_limit_bytes=96 * 1024 * 1024,
            disable_semaphore_checks=True,
        ),
    )(xt, w1.T, w2)

    out = out.reshape(H, CB, WT, SUB, LANES)
    out = jnp.transpose(out, (0, 1, 3, 2, 4)).reshape(1, H, C, W)
    return jnp.transpose(out, (0, 1, 3, 2))
```
